```python
import jax
import jax.numpy as jnp

def _softmax(x, axis=-1):
    return jax.nn.softmax(x, axis=axis)

def _gelu(x):
    return jax.nn.gelu(x, approximate=True)

def _silu(x):
    return jax.nn.silu(x)

def _sigmoid(x):
    return jax.nn.sigmoid(x)

def _layernorm(x, axis=-1, eps=1e-05):
    m = jnp.mean(x, axis=axis, keepdims=True)
    v = jnp.var(x, axis=axis, keepdims=True)
    return (x - m) / jnp.sqrt(v + eps)

def _scatter_add(tgt, idx, src, axis=0):
    return tgt.at[idx].add(src)

def _segment_sum(src, seg, n):
    return jax.ops.segment_sum(src, seg, n)

class _Rng:

    def __init__(self, key):
        self._k = key

    def _next(self):
        self._k, sub = jax.random.split(self._k)
        return sub

    def normal(self, shape):
        return jax.random.normal(self._next(), shape, dtype=jnp.bfloat16)

    def randint(self, lo, hi, shape):
        return jax.random.randint(self._next(), shape, lo, hi, dtype=jnp.int32)

    def uniform(self, shape, lo=0.0, hi=1.0):
        return jax.random.uniform(self._next(), shape, jnp.bfloat16, lo, hi)

    def permutation(self, n):
        return jax.random.permutation(self._next(), n)
kernel_name = 'gated_mix__memory_aug_recurrent_mem_tr__ssm_conv_h3__prompt'

def setup_inputs():
    _rng = _Rng(jax.random.key(int.from_bytes(__import__("os").urandom(4), "little")))
    _w = lambda a: (lambda t: t.astype(jnp.bfloat16) if jnp.issubdtype(t.dtype, jnp.floating) else t)(jnp.asarray(a))

    def _A_setup():
        B, S, Dm = (1, 2048, 640)
        H, Dh = (32, 192)
        M, seg = (8, 32)
        seg = min(seg, S)
        S = S // seg * seg
        return {'x': _w((lambda *s: _rng.normal(s) * 0.05)(B, S, Dm)), 'mem0': _w((lambda *s: _rng.normal(s) * 0.05)(B, M, Dm)), 'Wq': _w((lambda *s: _rng.normal(s) * 0.05)(Dm, H, Dh) * Dm ** (-0.5)), 'Wk': _w((lambda *s: _rng.normal(s) * 0.05)(Dm, H, Dh) * Dm ** (-0.5)), 'Wv': _w((lambda *s: _rng.normal(s) * 0.05)(Dm, H, Dh) * Dm ** (-0.5)), 'Wo': _w((lambda *s: _rng.normal(s) * 0.05)(H, Dh, Dm) * (H * Dh) ** (-0.5)), 'seg_len': seg}
    _A_in = _A_setup()

    def _B_setup():
        B, S, D = (1, 2048, 640)
        ks = 4
        return {'q': _w((lambda *s: _rng.normal(s) * 0.05)(B, S, D)), 'k': _w((lambda *s: _rng.normal(s) * 0.05)(B, S, D)), 'v': _w((lambda *s: _rng.normal(s) * 0.05)(B, S, D)), 'shift_k': _w((lambda *s: _rng.normal(s) * 0.05)(D, ks) * 0.5), 'ssm_k': _w((lambda *s: _rng.normal(s) * 0.05)(D, S) * (1.0 / S ** 0.5)), 'ssm_D': _w((lambda *s: _rng.normal(s) * 0.05)(D))}
    _B_in = _B_setup()
    return {'A_x': _A_in['x'], 'A_mem0': _A_in['mem0'], 'A_Wq': _A_in['Wq'], 'A_Wk': _A_in['Wk'], 'A_Wv': _A_in['Wv'], 'A_Wo': _A_in['Wo'], 'A_seg_len': _A_in['seg_len'], 'B_q': _B_in['q'], 'B_k': _B_in['k'], 'B_v': _B_in['v'], 'B_shift_k': _B_in['shift_k'], 'B_ssm_k': _B_in['ssm_k'], 'B_ssm_D': _B_in['ssm_D'], 'gate_w': _w((lambda *s: _rng.normal(s) * 0.05)(640))}

def reference(A_x, A_mem0, A_Wq, A_Wk, A_Wv, A_Wo, A_seg_len, B_q, B_k, B_v, B_shift_k, B_ssm_k, B_ssm_D, gate_w):

    def _A_ref(x, mem0, Wq, Wk, Wv, Wo, seg_len):
        B, S, Dm = x.shape
        H, Dh = (Wq.shape[1], Wq.shape[2])
        M = mem0.shape[1]
        scale = Dh ** (-0.5)
        n_seg = S // seg_len
        L = M + seg_len
        idx = jnp.arange(L)
        mask = (idx[:, None] < M) | (idx[:, None] >= idx[None, :])
        mem = mem0
        outs = []
        for s in range(n_seg):
            xs = x[:, s * seg_len:(s + 1) * seg_len, :].copy()
            h = jnp.concatenate([mem, xs], axis=1)
            q = jnp.einsum('btd,dhe->bhte', h, Wq)
            k = jnp.einsum('btd,dhe->bhte', h, Wk)
            v = jnp.einsum('btd,dhe->bhte', h, Wv)
            scores = jnp.einsum('bhqe,bhke->bhqk', q, k) * scale
            scores = jnp.where(mask[None, None], scores, -1000000000.0)
            p = _softmax(scores, axis=-1)
            o = jnp.einsum('bhqk,bhke->bhqe', p, v)
            o = jnp.einsum('bhte,hed->btd', o, Wo)
            mem = o[:, :M, :].copy()
            outs.append(o[:, M:, :])
        return jnp.concatenate(outs, axis=1)

    def _B_ref(q, k, v, shift_k, ssm_k, ssm_D):
        B, S, D = q.shape
        ks = shift_k.shape[-1]
        k_pad = jnp.pad(k, ((0, 0), (ks - 1, 0), (0, 0)))
        k_shift = jnp.zeros_like(k)
        for t in range(ks):
            k_shift = k_shift + k_pad[:, t:t + S, :] * shift_k[:, ks - 1 - t][None, None, :]
        kv = k_shift * v
        L = 2 * S
        kv_pad = jnp.pad(kv, ((0, 0), (0, S), (0, 0)))
        kf_pad = jnp.pad(ssm_k, ((0, 0), (0, S)))
        kv_f = (lambda x, axes=(-2, -1): jnp.fft.rfft2(x.astype(jnp.float32), axes=axes))(kv_pad[:, None, :, :], axes=(1, 2))
        kf_f = (lambda x, axes=(-2, -1): jnp.fft.rfft2(x.astype(jnp.float32), axes=axes))(kf_pad[:, None, :], axes=(1, 2))
        kf_f = (lambda x, *d: x.transpose(*d))(kf_f, 1, 2, 0)
        y_f = kv_f * kf_f[None, :, :, :]
        y = (lambda x, s, axes=(-2, -1): jnp.fft.irfft2(x, s=s, axes=axes).astype(jnp.bfloat16))(y_f, (1, L), axes=(1, 2))[:, 0, :S, :]
        y = y + kv * ssm_D[None, None, :]
        return q * y
    x = A_x
    g = _sigmoid((x * gate_w).sum(-1, keepdims=True))
    a = _A_ref(x, A_mem0, A_Wq, A_Wk, A_Wv, A_Wo, A_seg_len)
    b = _B_ref(x, B_k, B_v, B_shift_k, B_ssm_k, B_ssm_D)
    return g * a + (1 - g) * b
```

```python
import functools

import jax
import jax.numpy as jnp
import numpy as np
from jax import lax
from jax.experimental import pallas as pl
from jax.experimental.pallas import tpu as pltpu

F32 = jnp.float32
BF16 = jnp.bfloat16
NT = (((1,), (1,)), ((), ()))


def _dft_consts(C):
    k = np.arange(C)[:, None]
    n = np.arange(C)[None, :]
    ang = np.pi * (((2 * k + 1) * n) % (4 * C)) / (2 * C)
    fwd = np.concatenate([np.cos(ang), -np.sin(ang)], axis=0)
    inv = fwd.T / C
    return fwd.astype(jnp.bfloat16), inv.astype(jnp.bfloat16)


def make_kernel(S, D, H, Dh, M, seg, ks, C, opts):
    n_seg = S // seg
    L = M + seg
    HD = H * Dh
    PW = 2 * Dh
    NP = H // 2
    nb = S // C
    scale = float(Dh) ** -0.5
    WCH = opts.get('wch', 768)
    NWC = HD // WCH

    def kernel(x_hbm, mem0_ref, wq_hbm, wk_hbm, wv_hbm, wo_hbm, k_hbm, v_hbm, shift_ref, f_hbm,
               dvec_ref, gate_ref, fwd_ref, inv_ref,
               out_hbm,
               x_s, k_s, v_s, f_s, stage, w_s, wo_s, kf_s, kv_s, X_s, G_s, W_s, yb_s, out_s, mem_s,
               sem_in, sem_w, sem_out):
        cp_k = pltpu.make_async_copy(k_hbm, k_s, sem_in.at[0])
        cp_v = pltpu.make_async_copy(v_hbm, v_s, sem_in.at[1])
        cp_f = pltpu.make_async_copy(f_hbm, f_s, sem_in.at[2])
        cp_x = pltpu.make_async_copy(x_hbm, x_s, sem_in.at[3])
        cp_w = [[pltpu.make_async_copy(w.at[pl.ds(c * WCH, WCH), :], stage.at[i, pl.ds(c * WCH, WCH), :],
                                       sem_w.at[i * NWC + c])
                 for c in range(NWC)] for i, w in enumerate((wq_hbm, wk_hbm, wv_hbm, wo_hbm))]
        cp_f.start()
        cp_k.start()
        cp_v.start()
        for i in range(4):
            for c in range(NWC):
                cp_w[i][c].start()
        cp_x.start()

        if opts.get('do_b', True):
            fwd = fwd_ref[...]
            cp_f.wait()
            sgn = (1 - 2 * (lax.broadcasted_iota(jnp.int32, (C, D), 0) & 1)).astype(F32)
            prev = None
            for m in range(nb):
                fm = lax.dot_general(fwd, f_s[:, m * C:(m + 1) * C], NT, preferred_element_type=F32)
                if prev is None:
                    G_s[m] = fm
                else:
                    G_s[m, 0:C] = fm[0:C] - sgn * prev[C:2 * C]
                    G_s[m, C:2 * C] = fm[C:2 * C] + sgn * prev[0:C]
                prev = fm

            cp_k.wait()
            cp_v.wait()
            kf_s[0:8, :] = jnp.zeros((8, D), F32)
            kf_s[8:8 + S, :] = k_s[...].astype(F32)
            taps = shift_ref[...].astype(F32)
            for j in range(nb):
                acc = None
                for t in range(ks):
                    term = kf_s[8 - t + j * C:8 - t + (j + 1) * C, :] * taps[t:t + 1, :]
                    acc = term if acc is None else acc + term
                kv = (acc * v_s[j * C:(j + 1) * C, :].astype(F32)).astype(BF16)
                kv_s[j * C:(j + 1) * C, :] = kv
                X_s[j] = jnp.dot(fwd, kv, preferred_element_type=F32)

            RB = 16

            def freq_block(r, carry):
                r0 = pl.multiple_of(r * RB, RB)
                for c in range(D // 128):
                    cs = slice(c * 128, (c + 1) * 128)
                    xr = [X_s[j, pl.ds(r0, RB), cs] for j in range(nb)]
                    xi = [X_s[j, pl.ds(C + r0, RB), cs] for j in range(nb)]
                    gr = [G_s[j, pl.ds(r0, RB), cs] for j in range(nb)]
                    gi = [G_s[j, pl.ds(C + r0, RB), cs] for j in range(nb)]
                    for i in range(nb):
                        wr = wi = None
                        for j in range(i + 1):
                            tr = xr[j] * gr[i - j] - xi[j] * gi[i - j]
                            ti = xr[j] * gi[i - j] + xi[j] * gr[i - j]
                            wr = tr if wr is None else wr + tr
                            wi = ti if wi is None else wi + ti
                        W_s[i, pl.ds(r0, RB), cs] = wr.astype(BF16)
                        W_s[i, pl.ds(C + r0, RB), cs] = wi.astype(BF16)
                return carry

            lax.fori_loop(0, C // RB, freq_block, 0)

            inv = inv_ref[...]
            dvec = dvec_ref[...].astype(F32)
            for i in range(nb):
                y = jnp.dot(inv, W_s[i], preferred_element_type=F32)
                yb_s[i * C:(i + 1) * C, :] = y + kv_s[i * C:(i + 1) * C, :].astype(F32) * dvec
        else:
            cp_f.wait()
            cp_k.wait()
            cp_v.wait()
            yb_s[...] = jnp.zeros((S, D), F32)

        for i in range(3):
            for c in range(NWC):
                cp_w[i][c].wait()
                w_s[i, :, c * WCH:(c + 1) * WCH] = pltpu.bitcast(stage[i, c * WCH:(c + 1) * WCH, :].T, jnp.int32)
        for c in range(NWC):
            cp_w[3][c].wait()
            wo_s[c * WCH // 2:(c + 1) * WCH // 2, :] = pltpu.bitcast(stage[3, c * WCH:(c + 1) * WCH, :], jnp.int32)
        cp_x.wait()

        mem_s[...] = mem0_ref[...].astype(F32)
        gate = gate_ref[...].astype(F32)

        def step(s, carry):
            row = lax.broadcasted_iota(jnp.int32, (L, 128), 0)
            lane = lax.broadcasted_iota(jnp.int32, (L, 128), 1)
            first = lane < L
            second = (lane >= L) & (lane < 2 * L)
            key = jnp.where(first, lane, lane - L)
            visible = (row < M) | (row >= key)
            lo_half = lane < 64
            r0 = pl.multiple_of(s * seg, seg)
            xs = x_s[pl.ds(r0, seg), :].astype(F32)
            h = jnp.concatenate([mem_s[...], xs], axis=0)
            zeros = jnp.zeros((L, 128), F32)

            GP = 4
            GW = GP * PW
            NG = NP // GP

            def blockdiag(t0, t1, t2):
                top = jnp.concatenate([t0, jnp.where(lo_half, t1, 0.0), zeros], axis=1)
                bot = jnp.concatenate([zeros, jnp.where(lo_half, 0.0, t1), t2], axis=1)
                return jnp.concatenate([top, bot], axis=0).astype(BF16)

            def proj(i, G, j):
                c0 = G * GW + j * 512
                w = pltpu.bitcast(w_s[i, :, c0:c0 + 512], BF16)
                y = jnp.dot(h, w, preferred_element_type=F32)
                return [y[:, t * 128:(t + 1) * 128] for t in range(4)]

            def scores(q, kbd):
                if opts.get('kt', 'xpose') == 'xpose':
                    sc = lax.dot_general(q, kbd, NT, preferred_element_type=F32)
                    sc = jnp.concatenate([sc, jnp.zeros((L, 128 - 2 * L), F32)], axis=1)
                else:
                    kp = jnp.concatenate([kbd, jnp.zeros((128 - 2 * L, PW), BF16)], axis=0)
                    kt = kp.T
                    sc = jnp.dot(q, kt, preferred_element_type=F32)
                return sc

            def softmax(sc):
                sc = jnp.where(visible, sc * scale, -1e9)
                m1 = jnp.max(jnp.where(first, sc, -jnp.inf), axis=1, keepdims=True)
                m2 = jnp.max(jnp.where(second, sc, -jnp.inf), axis=1, keepdims=True)
                e = jnp.exp(sc - jnp.where(first, m1, m2))
                l1 = jnp.sum(jnp.where(first, e, 0.0), axis=1, keepdims=True)
                l2 = jnp.sum(jnp.where(second, e, 0.0), axis=1, keepdims=True)
                p = e / jnp.where(first, l1, l2)
                return p[:, 0:2 * L]

            qt, kt_, vt, pt, ot = {}, {}, {}, {}, {}
            accs = [None] * (D // 128)

            def do_q(G, j): qt.setdefault(G, []).extend(proj(0, G, j))
            def do_k(G, j): kt_.setdefault(G, []).extend(proj(1, G, j))
            def do_v(G, j): vt.setdefault(G, []).extend(proj(2, G, j))

            def do_s(G):
                pt[G] = []
                for p in range(GP):
                    q = jnp.concatenate(qt[G][3 * p:3 * p + 3], axis=1)
                    pt[G].append(softmax(scores(q, blockdiag(*kt_[G][3 * p:3 * p + 3]))))

            def do_pv(G):
                ot[G] = [jnp.dot(pt[G][p], blockdiag(*vt[G][3 * p:3 * p + 3]), preferred_element_type=F32)
                         for p in range(GP)]

            def do_o(G, j):
                for p in range(GP):
                    r0w = (G * GP + p) * PW // 2
                    w = pltpu.bitcast(wo_s[r0w:r0w + PW // 2, j * 128:(j + 1) * 128], BF16)
                    r = jnp.dot(ot[G][p], w, preferred_element_type=F32)
                    accs[j] = r if accs[j] is None else accs[j] + r

            sched = opts.get('sched', 0)
            if sched == 0:
                for G in range(NG):
                    for j in range(3): do_q(G, j)
                    for j in range(3): do_k(G, j)
                    if G > 0: do_pv(G - 1)
                    do_s(G)
                    for j in range(3): do_v(G, j)
                for G in range(NG):
                    if G == NG - 2: do_pv(NG - 1)
                    for j in range(5): do_o(G, j)
            elif sched == 1:
                for G in range(NG):
                    for j in range(3): do_q(G, j)
                    for j in range(3): do_k(G, j)
                    do_v(G, 0)
                    do_s(G)
                    do_v(G, 1); do_v(G, 2)
                    if G > 0:
                        for j in range(5): do_o(G - 1, j)
                    if G == NG - 1: pass
                    do_pv(G)
                for j in range(5): do_o(NG - 1, j)
            acc = jnp.concatenate(accs, axis=1)

            mem_s[...] = acc[0:M]
            a = acc[M:L]
            gsig = jax.nn.sigmoid(jnp.sum(xs * gate, axis=1, keepdims=True))
            b = xs * yb_s[pl.ds(r0, seg), :]
            out_s[pl.ds(r0, seg), :] = (gsig * a + (1.0 - gsig) * b).astype(BF16)
            pltpu.make_async_copy(out_s.at[pl.ds(r0, seg), :], out_hbm.at[pl.ds(r0, seg), :], sem_out.at[0]).start()
            return carry

        lax.fori_loop(0, n_seg, step, 0)
        pltpu.make_async_copy(out_s, out_hbm, sem_out.at[0]).wait()

    scratch = [
        pltpu.VMEM((S, D), BF16),
        pltpu.VMEM((S, D), BF16),
        pltpu.VMEM((S, D), BF16),
        pltpu.VMEM((D, S), BF16),
        pltpu.VMEM((4, HD, D), BF16),
        pltpu.VMEM((3, D // 2, HD), jnp.int32),
        pltpu.VMEM((HD // 2, D), jnp.int32),
        pltpu.VMEM((S + 8, D), F32),
        pltpu.VMEM((S, D), BF16),
        pltpu.VMEM((nb, 2 * C, D), F32),
        pltpu.VMEM((nb, 2 * C, D), F32),
        pltpu.VMEM((nb, 2 * C, D), BF16),
        pltpu.VMEM((S, D), F32),
        pltpu.VMEM((S, D), BF16),
        pltpu.VMEM((M, D), F32),
        pltpu.SemaphoreType.DMA((5,)),
        pltpu.SemaphoreType.DMA((4 * NWC,)),
        pltpu.SemaphoreType.DMA((1,)),
    ]
    return kernel, scratch


_OPTS = {'sched': 1}


@functools.partial(jax.jit, static_argnames=("A_seg_len",))
def pallas_gated_mix__memory_aug_recurrent_mem_tr__ssm_conv_h3__prompt_kernel(
    A_x, A_mem0, A_Wq, A_Wk, A_Wv, A_Wo, A_seg_len, B_q, B_k, B_v, B_shift_k, B_ssm_k, B_ssm_D, gate_w,
):
    opts = _OPTS
    B, S, D = A_x.shape
    H, Dh = A_Wq.shape[1], A_Wq.shape[2]
    M = A_mem0.shape[1]
    seg = int(A_seg_len)
    ks = B_shift_k.shape[1]
    C = opts.get('C', 256)
    fwd, inv = _dft_consts(C)
    kernel, scratch = make_kernel(S, D, H, Dh, M, seg, ks, C, opts)
    wt = lambda w: jnp.transpose(w, (1, 2, 0)).reshape(H * Dh, D)
    hbm = pl.BlockSpec(memory_space=pl.ANY)
    vmem = pl.BlockSpec(memory_space=pltpu.VMEM)
    out = pl.pallas_call(
        kernel,
        out_shape=jax.ShapeDtypeStruct((S, D), BF16),
        in_specs=[hbm, vmem, hbm, hbm, hbm, hbm, hbm, hbm, vmem, hbm, vmem, vmem, vmem, vmem],
        out_specs=hbm,
        scratch_shapes=scratch,
        compiler_params=pltpu.CompilerParams(vmem_limit_bytes=120 * 1024 * 1024, **opts.get('cp', {})),
    )(A_x.reshape(S, D), A_mem0.reshape(M, D), wt(A_Wq), wt(A_Wk), wt(A_Wv), A_Wo.reshape(H * Dh, D),
      B_k.reshape(S, D), B_v.reshape(S, D), B_shift_k.T, B_ssm_k,
      B_ssm_D.reshape(1, D), gate_w.reshape(1, D), fwd, inv)
    return out.reshape(B, S, D)
```

```python
import contextlib
import functools

import jax
import jax.numpy as jnp
import numpy as np
from jax import lax
from jax.experimental import pallas as pl
from jax.experimental.pallas import tpu as pltpu

F32 = jnp.float32
BF16 = jnp.bfloat16
NT = (((1,), (1,)), ((), ()))


def _pack_rows(a):
    u = np.ascontiguousarray(a.astype(jnp.bfloat16)).view(np.uint16).astype(np.uint32)
    return (u[0::2] | (u[1::2] << 16)).view(np.int32)


def _dft_consts(C):
    k = np.concatenate([np.arange(0, C, 2), np.arange(1, C, 2)])[:, None]
    n = np.arange(C)[None, :]
    ang = np.pi * (((2 * k + 1) * n) % (4 * C)) / (2 * C)
    fwd = np.concatenate([np.cos(ang), -np.sin(ang)], axis=0)
    inv = fwd.T / C
    return _pack_rows(fwd), _pack_rows(inv)


def make_sched(kind, NG):
    if not isinstance(kind, int):
        return kind.split()
    q = lambda G: [f'q{G}{j}' for j in range(3)]
    k = lambda G: [f'k{G}{j}' for j in range(3)]
    v = lambda G: [f'v{G}{j}' for j in range(3)]
    o = lambda G: [f'o{G}{j}' for j in range(5)]
    out = []
    if kind == 1:
        for G in range(NG):
            out += q(G) + k(G) + v(G)[:1] + [f's{G}'] + v(G)[1:]
            if G > 0: out += o(G - 1)
            out += [f'p{G}']
        out += o(NG - 1)
    elif kind == 2:
        for G in range(NG):
            out += q(G)
            if G > 0: out += [f'p{G-1}']
            out += k(G) + v(G)[:1] + [f's{G}'] + v(G)[1:]
            if G > 0: out += o(G - 1)
        out += [f'p{NG-1}'] + o(NG - 1)
    elif kind == 3:
        for G in range(NG):
            out += q(G)
            if G > 0: out += [f'p{G-1}']
            out += k(G) + v(G)[:1] + [f's{G}'] + v(G)[1:]
        for G in range(NG):
            if G == NG - 1: out += [f'p{G}']
            out += o(G)
    elif kind == 4:
        for G in range(NG):
            out += q(G)
            if G > 0: out += [f'p{G-1}']
            out += k(G) + v(G)[:1] + [f's{G}'] + v(G)[1:]
            if G > 1: out += o(G - 2)
        out += o(NG - 2) + [f'p{NG-1}'] + o(NG - 1)
    return out


def make_kernel(S, D, H, Dh, M, seg, ks, C, opts):
    n_seg = S // seg
    L = M + seg
    HD = H * Dh
    PW = 2 * Dh
    NP = H // 2
    nb = S // C
    scale = float(Dh) ** -0.5
    CW = 512
    NC = HD // CW
    NPRE = opts.get('npre', 16)
    NF = 16
    RB = opts.get('rb', 16)
    DW = opts.get('dw', 1536)
    ND = HD // DW
    scope = jax.named_scope if opts.get('scopes') else (lambda name: contextlib.nullcontext())

    def kernel(x_hbm, mem0_ref, wq_hbm, wk_hbm, wv_hbm, wo_hbm, k_hbm, v_hbm, shift_ref, f_hbm,
               dvec_ref, gate_ref, fwd_ref, inv_ref,
               out_hbm,
               x_s, k_s, v_s, f_s, stage, w_s, wo_s, kf_s, X_s, F_s, W_s, xl_s, pre_s, mem_s,
               sem_in, sem_f, sem_kv, sem_w, sem_out):
        vec = (lambda r: r[...].astype(F32).reshape(1, D)) if opts.get('oned') else (lambda r: r[...].astype(F32))
        out_s = k_s
        if opts.get('inplace'):
            W_s = X_s
        KP = opts.get('kp', 2)
        KR = S // KP

        def kv_copy(p):
            rows = pl.ds(p * KR, KR)
            return (pltpu.make_async_copy(k_hbm.at[rows, :], k_s.at[rows, :], sem_kv.at[2 * p]),
                    pltpu.make_async_copy(v_hbm.at[rows, :], v_s.at[rows, :], sem_kv.at[2 * p + 1]))

        FPS = opts.get('fp', (0, 2, 8))
        cp_f = [pltpu.make_async_copy(f_hbm.at[:, pl.ds(a * C, (b - a) * C)], f_s.at[:, pl.ds(a * C, (b - a) * C)],
                                      sem_f.at[p]) for p, (a, b) in enumerate(zip(FPS[:-1], FPS[1:]))]
        cp_x = pltpu.make_async_copy(x_hbm, x_s, sem_in.at[0])
        w_hbm = (wq_hbm, wk_hbm, wv_hbm, wo_hbm)

        def w_copy(i, d):
            return pltpu.make_async_copy(w_hbm[i].at[pl.ds(d * DW, DW), :],
                                         stage.at[i, pl.ds(d * DW, DW), :], sem_w.at[i * ND + d])

        def wait_chunk(n):
            per = DW // CW

            @pl.when(n % per == 0)
            def _():
                pltpu.make_async_copy(wq_hbm.at[pl.ds(0, DW), :], stage.at[0, pl.ds(0, DW), :],
                                      sem_w.at[n // per]).wait()

        def flip(n):
            i = n // NC
            c0 = pl.multiple_of((n % NC) * CW, CW)
            w_s[i, :, pl.ds(c0, CW)] = pltpu.bitcast(stage[i, pl.ds(c0, CW), :].T, jnp.int32)

        def project_ahead(n):
            i = n // NC
            c0 = pl.multiple_of((n % NC) * CW, CW)
            xl = pltpu.bitcast(xl_s[...], BF16)
            pre_s[n] = lax.dot_general(xl, stage[i, pl.ds(c0, CW), :], NT, preferred_element_type=F32)

        loads = []
        for name in opts.get('dma', 'f k x 0 1 2 3').split():
            if name == 'f': loads += cp_f
            elif name == 'x': loads += [cp_x]
            elif name == 'k': loads += [cp for p in range(KP) for cp in kv_copy(p)]
            else: loads += [w_copy(int(name), d) for d in range(ND)]

        def issue(n, carry):
            for idx, cp in enumerate(loads):
                pl.when(n == idx)(cp.start)
            return carry

        lax.fori_loop(0, len(loads), issue, 0)


        def filt(m, carry):
            c0 = pl.multiple_of(m * C, C)
            F_s[m] = lax.dot_general(pltpu.bitcast(fwd_ref[...], BF16), f_s[:, pl.ds(c0, C)], NT,
                                     preferred_element_type=F32)
            return carry

        UB = opts.get('ub', 2)
        with scope('filt'):
            for p, (a, b) in enumerate(zip(FPS[:-1], FPS[1:])):
                cp_f[p].wait()
                lax.fori_loop(a, b, filt, 0, unroll=min(UB, b - a))
        kf_s[0:8, :] = jnp.zeros((8, D), F32)

        def sig(j, carry):
            r0 = pl.multiple_of(j * C, C)
            taps = shift_ref[...].astype(F32)
            kc = k_s[pl.ds(r0, C), :].astype(F32)
            if opts.get('shift', 'mem') == 'mem':
                kf_s[8:8 + C, :] = kc
                acc = kc * taps[0:1, :]
                for t in range(1, ks):
                    acc = acc + kf_s[8 - t:8 - t + C, :] * taps[t:t + 1, :]
                kf_s[0:8, :] = kc[C - 8:C]
            else:
                ext = jnp.concatenate([kf_s[0:8, :], kc], axis=0)
                acc = kc * taps[0:1, :]
                for t in range(1, ks):
                    acc = acc + pltpu.roll(ext, t, 0)[8:8 + C] * taps[t:t + 1, :]
                kf_s[0:8, :] = kc[C - 8:C]
            kv = (acc * v_s[pl.ds(r0, C), :].astype(F32)).astype(BF16)
            v_s[pl.ds(r0, C), :] = kv
            X_s[j] = jnp.dot(pltpu.bitcast(fwd_ref[...], BF16), kv, preferred_element_type=F32)
            return carry

        with scope('sig'):
            for p in range(KP):
                for cp in kv_copy(p):
                    cp.wait()
                lax.fori_loop(p * nb // KP, (p + 1) * nb // KP, sig, 0, unroll=UB)

        def freq_block(r, carry, odd):
            r0 = pl.multiple_of(r * RB, RB)
            for c in range(D // 128):
                cs = slice(c * 128, (c + 1) * 128)
                xr = [X_s[j, pl.ds(r0, RB), cs] for j in range(nb)]
                xi = [X_s[j, pl.ds(C + r0, RB), cs] for j in range(nb)]
                fr = [F_s[j, pl.ds(r0, RB), cs] for j in range(nb)]
                fi = [F_s[j, pl.ds(C + r0, RB), cs] for j in range(nb)]
                if odd:
                    gr = [fr[0]] + [fr[m] + fi[m - 1] for m in range(1, nb)]
                    gi = [fi[0]] + [fi[m] - fr[m - 1] for m in range(1, nb)]
                else:
                    gr = [fr[0]] + [fr[m] - fi[m - 1] for m in range(1, nb)]
                    gi = [fi[0]] + [fi[m] + fr[m - 1] for m in range(1, nb)]
                if opts.get('gauss'):
                    xs_ = [a + b for a, b in zip(xr, xi)]
                    gd = [b - a for a, b in zip(gr, gi)]
                    gs = [a + b for a, b in zip(gr, gi)]
                for i in range(nb):
                    if opts.get('gauss'):
                        k1 = k2 = k3 = None
                        for j in range(i + 1):
                            t1, t2, t3 = gr[i - j] * xs_[j], xr[j] * gd[i - j], xi[j] * gs[i - j]
                            k1, k2, k3 = (t1, t2, t3) if j == 0 else (k1 + t1, k2 + t2, k3 + t3)
                        wr, wi = k1 - k3, k1 + k2
                    else:
                        wr = wi = None
                        for j in range(i + 1):
                            tr = xr[j] * gr[i - j] - xi[j] * gi[i - j]
                            ti = xr[j] * gi[i - j] + xi[j] * gr[i - j]
                            wr = tr if wr is None else wr + tr
                            wi = ti if wi is None else wi + ti
                    W_s[i, pl.ds(r0, RB), cs] = wr.astype(W_s.dtype)
                    W_s[i, pl.ds(C + r0, RB), cs] = wi.astype(W_s.dtype)
            return carry

        with scope('freq'):
            lax.fori_loop(0, C // RB // 2, functools.partial(freq_block, odd=False), 0)
            lax.fori_loop(C // RB // 2, C // RB, functools.partial(freq_block, odd=True), 0)

        def inverse(i, carry):
            r0 = pl.multiple_of(i * C, C)
            y = jnp.dot(pltpu.bitcast(inv_ref[...], BF16), W_s[i].astype(BF16), preferred_element_type=F32)
            dvec = vec(dvec_ref)
            v_s[pl.ds(r0, C), :] = (y + v_s[pl.ds(r0, C), :].astype(F32) * dvec).astype(BF16)
            return carry

        with scope('inverse'):
            lax.fori_loop(0, nb, inverse, 0, unroll=UB)

        cp_x.wait()

        def last_rows(s2, carry):
            r0 = pl.multiple_of(s2 * 2 * seg, 2 * seg)
            lo = x_s[pl.ds(r0 + seg - 16, 16), :].astype(F32)[8:16]
            hi = x_s[pl.ds(r0 + 2 * seg - 16, 16), :].astype(F32)[8:16]
            xl_s[pl.ds(pl.multiple_of(s2 * 8, 8), 8), :] = pltpu.bitcast(
                jnp.concatenate([lo, hi], axis=0).astype(BF16), jnp.int32)
            return carry

        lax.fori_loop(0, n_seg // 2, last_rows, 0, unroll=4)

        def ahead(n, carry, base, nflip):
            for e in range(nflip):
                wait_chunk(base + nflip * n + e)
            project_ahead(n)
            for e in range(nflip):
                flip(base + nflip * n + e)
            return carry

        def flip_rest(n, carry):
            wait_chunk(n)
            flip(n)
            return carry

        hi = -(-3 * NC // NPRE)
        n_lo = hi * NPRE - 3 * NC
        with scope('ahead1'):
            if n_lo:
                lax.fori_loop(0, n_lo, functools.partial(ahead, base=0, nflip=hi - 1), 0, unroll=opts.get('ua', 1))
        with scope('ahead2'):
            lax.fori_loop(n_lo, NPRE, functools.partial(ahead, base=-n_lo, nflip=hi), 0, unroll=opts.get('ua', 1))

        def pack(d, carry):
            r0 = pl.multiple_of(d * DW, DW)
            h0 = pl.multiple_of(d * (DW // 2), DW // 2)
            pltpu.make_async_copy(wo_hbm.at[pl.ds(0, DW), :], stage.at[0, pl.ds(0, DW), :],
                                  sem_w.at[3 * ND + d]).wait()
            wo_s[pl.ds(h0, DW // 2), :] = pltpu.bitcast(stage[3, pl.ds(r0, DW), :], jnp.int32)
            return carry

        with scope('pack'):
            lax.fori_loop(0, ND, pack, 0)

        mem_s[...] = mem0_ref[...].astype(F32)
        gate = vec(gate_ref)

        def step(s, carry):
            row = lax.broadcasted_iota(jnp.int32, (L, 128), 0)
            lane = lax.broadcasted_iota(jnp.int32, (L, 128), 1)
            first = lane < L
            second = (lane >= L) & (lane < 2 * L)
            key = jnp.where(first, lane, lane - L)
            visible = (row < M) | (row >= key)
            lo_half = lane < 64
            r0 = pl.multiple_of(s * seg, seg)
            p0 = pl.multiple_of(s * 8, 8)
            xs = x_s[pl.ds(r0, seg), :].astype(F32)
            h = jnp.concatenate([mem_s[...], xs], axis=0)
            zeros = jnp.zeros((L, 128), F32)

            GP = 4
            GW = GP * PW
            NG = NP // GP

            def blockdiag(t0, t1, t2):
                top = jnp.concatenate([t0, jnp.where(lo_half, t1, 0.0), zeros], axis=1)
                bot = jnp.concatenate([zeros, jnp.where(lo_half, 0.0, t1), t2], axis=1)
                return jnp.concatenate([top, bot], axis=0).astype(BF16)

            def proj(i, G, j):
                c0 = G * GW + j * 512
                w = pltpu.bitcast(w_s[i, :, c0:c0 + 512], BF16)
                n = i * NC + c0 // CW
                if n < NPRE:
                    y = jnp.dot(h[0:L - 8], w, preferred_element_type=F32)
                    y = jnp.concatenate([y, pre_s[n, pl.ds(p0, 8), :]], axis=0)
                else:
                    y = jnp.dot(h, w, preferred_element_type=F32)
                return [y[:, t * 128:(t + 1) * 128] for t in range(4)]

            def scores(q, kbd):
                if opts.get('kt', 'xpose') == 'xpose':
                    sc = lax.dot_general(q, kbd, NT, preferred_element_type=F32)
                    sc = jnp.concatenate([sc, jnp.zeros((L, 128 - 2 * L), F32)], axis=1)
                else:
                    kp = jnp.concatenate([kbd, jnp.zeros((128 - 2 * L, PW), BF16)], axis=0)
                    kt = kp.T
                    sc = jnp.dot(q, kt, preferred_element_type=F32)
                return sc

            def softmax(sc):
                sc = jnp.where(visible, sc * scale, -1e9)
                m1 = jnp.max(jnp.where(first, sc, -jnp.inf), axis=1, keepdims=True)
                m2 = jnp.max(jnp.where(second, sc, -jnp.inf), axis=1, keepdims=True)
                e = jnp.exp(sc - jnp.where(first, m1, m2))
                l1 = jnp.sum(jnp.where(first, e, 0.0), axis=1, keepdims=True)
                l2 = jnp.sum(jnp.where(second, e, 0.0), axis=1, keepdims=True)
                p = e / jnp.where(first, l1, l2)
                return p[:, 0:2 * L]

            qt, kt_, vt, pt, ot = {}, {}, {}, {}, {}
            accs = [None] * (D // 128)

            def do_q(G, j): qt.setdefault(G, []).extend(proj(0, G, j))
            def do_k(G, j): kt_.setdefault(G, []).extend(proj(1, G, j))
            def do_v(G, j): vt.setdefault(G, []).extend(proj(2, G, j))

            def do_s(G):
                pt[G] = []
                for p in range(GP):
                    q = jnp.concatenate(qt[G][3 * p:3 * p + 3], axis=1)
                    pt[G].append(softmax(scores(q, blockdiag(*kt_[G][3 * p:3 * p + 3]))))

            def do_pv(G):
                ot[G] = [jnp.dot(pt[G][p], blockdiag(*vt[G][3 * p:3 * p + 3]), preferred_element_type=F32)
                         for p in range(GP)]

            def do_o(G, j):
                for p in range(GP):
                    r0w = (G * GP + p) * PW // 2
                    w = pltpu.bitcast(wo_s[r0w:r0w + PW // 2, j * 128:(j + 1) * 128], BF16)
                    r = jnp.dot(ot[G][p], w, preferred_element_type=F32)
                    accs[j] = r if accs[j] is None else accs[j] + r

            for op in make_sched(opts.get('sched', 1), NG):
                kind, G = op[0], int(op[1])
                if kind == 'q': do_q(G, int(op[2]))
                elif kind == 'k': do_k(G, int(op[2]))
                elif kind == 'v': do_v(G, int(op[2]))
                elif kind == 's': do_s(G)
                elif kind == 'p': do_pv(G)
                elif kind == 'o': do_o(G, int(op[2]))
            acc = jnp.concatenate(accs, axis=1)

            mem_s[...] = acc[0:M]
            a = acc[M:L]
            gsig = jax.nn.sigmoid(jnp.sum(xs * gate, axis=1, keepdims=True))
            b = xs * v_s[pl.ds(r0, seg), :].astype(F32)
            out_s[pl.ds(r0, seg), :] = (gsig * a + (1.0 - gsig) * b).astype(BF16)
            pltpu.make_async_copy(out_s.at[pl.ds(r0, seg), :], out_hbm.at[pl.ds(r0, seg), :], sem_out.at[0]).start()
            return carry

        with scope('main'):
            lax.fori_loop(0, opts.get('nsteps', n_seg), step, 0, unroll=opts.get('unroll', 1))
        _n = opts.get('nsteps', n_seg) * seg; pltpu.make_async_copy(out_s.at[pl.ds(0, _n), :], out_hbm.at[pl.ds(0, _n), :], sem_out.at[0]).wait()

    scratch = [
        pltpu.VMEM((S, D), BF16),
        pltpu.VMEM((S, D), BF16),
        pltpu.VMEM((S, D), BF16),
        pltpu.VMEM((D, S), BF16),
        pltpu.VMEM((4, HD, D), BF16),
        pltpu.VMEM((3, D // 2, HD), jnp.int32),
        pltpu.VMEM((HD // 2, D), jnp.int32),
        pltpu.VMEM((C + 8, D), F32),
        pltpu.VMEM((nb, 2 * C, D), F32),
        pltpu.VMEM((nb, 2 * C, D), F32),
        pltpu.VMEM((8, 128) if opts.get('inplace') else (nb, 2 * C, D), BF16 if RB % 16 == 0 else F32),
        pltpu.VMEM((n_seg * 4, D), jnp.int32),
        pltpu.VMEM((NPRE, n_seg * 8, CW), F32),
        pltpu.VMEM((M, D), F32),
        pltpu.SemaphoreType.DMA((1,)),
        pltpu.SemaphoreType.DMA((len(opts.get('fp', (0, 2, 8))) - 1,)),
        pltpu.SemaphoreType.DMA((2 * opts.get('kp', 2),)),
        pltpu.SemaphoreType.DMA((4 * ND,)),
        pltpu.SemaphoreType.DMA((1,)),
    ]
    return kernel, scratch


_OPTS = {'sched':2,'C':256,'gauss':True,'rb':8,'inplace':True,'oned':True,'ub':4,'ua':2,'npre':12,'unroll':2}


@functools.partial(jax.jit, static_argnames=("A_seg_len",))
def pallas_gated_mix__memory_aug_recurrent_mem_tr__ssm_conv_h3__prompt_kernel(
    A_x, A_mem0, A_Wq, A_Wk, A_Wv, A_Wo, A_seg_len, B_q, B_k, B_v, B_shift_k, B_ssm_k, B_ssm_D, gate_w,
):
    opts = _OPTS
    B, S, D = A_x.shape
    H, Dh = A_Wq.shape[1], A_Wq.shape[2]
    M = A_mem0.shape[1]
    seg = int(A_seg_len)
    ks = B_shift_k.shape[1]
    C = opts.get('C', 256)
    fwd, inv = _dft_consts(C)
    kernel, scratch = make_kernel(S, D, H, Dh, M, seg, ks, C, opts)
    wt = lambda w: jnp.transpose(w, (1, 2, 0)).reshape(H * Dh, D)
    hbm = pl.BlockSpec(memory_space=pl.ANY)
    vmem = pl.BlockSpec(memory_space=pltpu.VMEM)
    out = pl.pallas_call(
        kernel,
        out_shape=jax.ShapeDtypeStruct((S, D), BF16),
        in_specs=[hbm, vmem, hbm, hbm, hbm, hbm, hbm, hbm, vmem, hbm, vmem, vmem, vmem, vmem],
        out_specs=hbm,
        scratch_shapes=scratch,
        compiler_params=pltpu.CompilerParams(vmem_limit_bytes=126 * 1024 * 1024, **opts.get('cp', {})),
    )(A_x.reshape(S, D), A_mem0.reshape(M, D), wt(A_Wq), wt(A_Wk), wt(A_Wv), A_Wo.reshape(H * Dh, D),
      B_k.reshape(S, D), B_v.reshape(S, D), B_shift_k.T, B_ssm_k,
      *((B_ssm_D, gate_w) if opts.get('oned') else (B_ssm_D.reshape(1, D), gate_w.reshape(1, D))), fwd, inv)
    return out.reshape(B, S, D)
```

```python
import contextlib
import functools

import jax
import jax.numpy as jnp
import numpy as np
from jax import lax
from jax.experimental import pallas as pl
from jax.experimental.pallas import tpu as pltpu

F32 = jnp.float32
BF16 = jnp.bfloat16
I32 = jnp.int32
NT = (((1,), (1,)), ((), ()))
LANES = 128


def _pack_rows(a):
    u = np.ascontiguousarray(a.astype(jnp.bfloat16)).view(np.uint16).astype(np.uint32)
    return (u[0::2] | (u[1::2] << 16)).view(np.int32)


def _dft_consts(C):
    k = np.concatenate([np.arange(0, C, 2), np.arange(1, C, 2)])[:, None]
    n = np.arange(C)[None, :]
    ang = np.pi * (((2 * k + 1) * n) % (4 * C)) / (2 * C)
    full = np.concatenate([np.cos(ang), -np.sin(ang)], axis=0)
    u = np.arange(C // 2)[None, :]
    ang = np.pi * (((2 * k + 1) * (2 * u + 1)) % (8 * C)) / (4 * C)
    half = np.concatenate([np.cos(ang), -np.sin(ang)], axis=0)
    inv = half.T / C
    return _pack_rows(full), _pack_rows(half), _pack_rows(inv)


def _unpack(a):
    return pltpu.bitcast(a, BF16)


def _pack(a):
    return pltpu.bitcast(a, I32)


def _reverse_rows(a):
    idx = 7 - lax.broadcasted_iota(I32, (8, a.shape[1]), 0)
    return jnp.concatenate(
        [jnp.take_along_axis(a[r:r + 8], idx, axis=0) for r in range(a.shape[0] - 8, -8, -8)], axis=0)


def make_sched(kind, NG):
    if not isinstance(kind, int):
        return kind.split()
    q = lambda G: [f'q{G}{j}' for j in range(3)]
    k = lambda G: [f'k{G}{j}' for j in range(3)]
    v = lambda G: [f'v{G}{j}' for j in range(3)]
    o = lambda G: [f'o{G}{j}' for j in range(5)]
    out = []
    if kind == 2:
        for G in range(NG):
            out += q(G)
            if G > 0: out += [f'p{G-1}']
            out += k(G) + v(G)[:1] + [f's{G}'] + v(G)[1:]
            if G > 0: out += o(G - 1)
        out += [f'p{NG-1}'] + o(NG - 1)
    return out


def make_kernel(S, D, H, Dh, M, seg, ks, C, opts):
    n_seg = S // seg
    L = M + seg
    HD = H * Dh
    PW = 2 * Dh
    nb = S // C
    scale = float(Dh) ** -0.5
    CW = 4 * LANES
    NC = HD // CW
    GP = 4
    NG = H // 2 // GP
    DW = 3 * CW
    ND = HD // DW
    UA = opts.get('ua', 3)
    FLIPS = opts.get('flips', (1, 2, 3, 3, 3))
    NPRE = UA * len(FLIPS)
    FPS = opts.get('fp', (0, 2, 8))
    KP = opts.get('kp', 2)
    assert PW == 3 * LANES and 2 * L <= LANES and M == 8 and seg % 16 == 0 and sum(FLIPS) == 3 * ND
    scope = jax.named_scope if opts.get('scopes') else (lambda name: contextlib.nullcontext())

    def kernel(x_hbm, mem0_ref, wq_hbm, wk_hbm, wv_hbm, wo_hbm, k_hbm, v_hbm, shift_ref, f_hbm,
               dvec_ref, gate_ref, full_ref, half_ref, inv_ref,
               out_hbm,
               x_s, k_s, v_s, f_s, stage, w_s, tail_s, X_s, F_s, W_s, xl_s, pre_s, mem_s,
               sem_x, sem_f, sem_kv, sem_w, sem_out):
        out_s = k_s

        cp_x = pltpu.make_async_copy(x_hbm, x_s, sem_x.at[0])
        cp_f = [pltpu.make_async_copy(f_hbm.at[:, pl.ds(a * C, (b - a) * C)],
                                      f_s.at[:, pl.ds(a * C, (b - a) * C)], sem_f.at[p])
                for p, (a, b) in enumerate(zip(FPS[:-1], FPS[1:]))]
        cp_kv = [[pltpu.make_async_copy(src.at[pl.ds(p * S // KP, S // KP), :],
                                        dst.at[pl.ds(p * S // KP, S // KP), :], sem_kv.at[2 * p + e])
                  for e, (src, dst) in enumerate(((k_hbm, k_s), (v_hbm, v_s)))] for p in range(KP)]
        cp_w = [pltpu.make_async_copy(w.at[pl.ds(d * DW, DW), :], stage.at[i, pl.ds(d * DW, DW), :],
                                      sem_w.at[i * ND + d])
                for i, w in enumerate((wq_hbm, wk_hbm, wv_hbm, wo_hbm)) for d in range(ND)]
        loads = cp_f + sum(cp_kv, []) + [cp_x] + cp_w

        def issue(n, carry):
            for idx, cp in enumerate(loads):
                pl.when(n == idx)(cp.start)
            return carry

        lax.fori_loop(0, len(loads), issue, 0)

        def filt(m, carry):
            c0 = pl.multiple_of(m * C, C)
            F_s[m] = lax.dot_general(_unpack(full_ref[...]), f_s[:, pl.ds(c0, C)], NT, preferred_element_type=F32)
            return carry

        with scope('filt'):
            for p, (a, b) in enumerate(zip(FPS[:-1], FPS[1:])):
                cp_f[p].wait()
                lax.fori_loop(a, b, filt, 0, unroll=min(opts.get('ub', 2), b - a))

        def delay(a, n, slot):
            tail = tail_s[slot]
            tail_s[slot] = a[a.shape[0] - 8:]
            rolled = [pltpu.roll(g, n, 0) for g in [tail] + [a[r:r + 8] for r in range(0, a.shape[0], 8)]]
            early = lax.broadcasted_iota(I32, tail.shape, 0) < n
            return jnp.concatenate([jnp.where(early, p, c) for p, c in zip(rolled[:-1], rolled[1:])], axis=0)

        def sig(j, carry):
            r0 = pl.multiple_of(j * C, C)
            taps = shift_ref[...].astype(F32)
            kc = k_s[pl.ds(r0, C), :].astype(F32)
            k1 = delay(kc, 1, 0)
            acc = None
            for p in range((ks + 1) // 2):
                pair = kc * taps[2 * p:2 * p + 1, :]
                if 2 * p + 1 < ks:
                    pair = pair + k1 * taps[2 * p + 1:2 * p + 2, :]
                acc = pair if p == 0 else acc + delay(pair, 2 * p, p)
            kv = acc * v_s[pl.ds(r0, C), :].astype(F32)
            v_s[pl.ds(r0, C), :] = kv.astype(BF16)
            up, down = kv[C // 2:C], _reverse_rows(kv[0:C // 2])
            X_s[j, 0:C] = jnp.dot(_unpack(half_ref[0:C // 2, :]), (up + down).astype(BF16),
                                  preferred_element_type=F32)
            X_s[j, C:2 * C] = jnp.dot(_unpack(half_ref[C // 2:C, :]), (up - down).astype(BF16),
                                      preferred_element_type=F32)
            return carry

        tail_s[...] = jnp.zeros(tail_s.shape, F32)
        with scope('sig'):
            for p in range(KP):
                for cp in cp_kv[p]:
                    cp.wait()
                lax.fori_loop(p * nb // KP, (p + 1) * nb // KP, sig, 0, unroll=opts.get('us', 2))

        def freq(r, carry, odd):
            re = pl.ds(pl.multiple_of(r * 8, 8), 8)
            im = pl.ds(pl.multiple_of(C + r * 8, 8), 8)
            for c in range(D // LANES):
                cs = slice(c * LANES, (c + 1) * LANES)
                xr = [X_s[j, re, cs] for j in range(nb)]
                xi = [X_s[j, im, cs] for j in range(nb)]
                fr = [F_s[j, re, cs] for j in range(nb)]
                fi = [F_s[j, im, cs] for j in range(nb)]
                if odd:
                    gr = [fr[0]] + [fr[m] + fi[m - 1] for m in range(1, nb)]
                    gi = [fi[0]] + [fi[m] - fr[m - 1] for m in range(1, nb)]
                else:
                    gr = [fr[0]] + [fr[m] - fi[m - 1] for m in range(1, nb)]
                    gi = [fi[0]] + [fi[m] + fr[m - 1] for m in range(1, nb)]
                xs = [a + b for a, b in zip(xr, xi)]
                gd = [b - a for a, b in zip(gr, gi)]
                gs = [a + b for a, b in zip(gr, gi)]
                for i in range(nb):
                    k1 = k2 = k3 = None
                    for j in range(i + 1):
                        t1, t2, t3 = gr[i - j] * xs[j], xr[j] * gd[i - j], xi[j] * gs[i - j]
                        k1, k2, k3 = (t1, t2, t3) if j == 0 else (k1 + t1, k2 + t2, k3 + t3)
                    W_s[i, re, cs] = k1 - k3
                    W_s[i, im, cs] = k1 + k2
            return carry

        with scope('freq'):
            lax.fori_loop(0, C // 16, functools.partial(freq, odd=False), 0)
            lax.fori_loop(C // 16, C // 8, functools.partial(freq, odd=True), 0)

        def inverse(i, carry):
            r0 = pl.multiple_of(i * C, C)
            even = jnp.dot(_unpack(inv_ref[:, 0:C]), W_s[i, 0:C].astype(BF16), preferred_element_type=F32)
            odd = jnp.dot(_unpack(inv_ref[:, C:2 * C]), W_s[i, C:2 * C].astype(BF16), preferred_element_type=F32)
            y = jnp.concatenate([_reverse_rows(even - odd), even + odd], axis=0)
            dvec = dvec_ref[...].astype(F32).reshape(1, D)
            v_s[pl.ds(r0, C), :] = (y + v_s[pl.ds(r0, C), :].astype(F32) * dvec).astype(BF16)
            return carry

        with scope('inverse'):
            lax.fori_loop(0, nb, inverse, 0, unroll=opts.get('ui', 2))

        cp_x.wait()

        def last_rows(s2, carry):
            r0 = pl.multiple_of(s2 * 2 * seg, 2 * seg)
            lo = x_s[pl.ds(r0 + seg - 16, 16), :].astype(F32)[8:16]
            hi = x_s[pl.ds(r0 + 2 * seg - 16, 16), :].astype(F32)[8:16]
            xl_s[pl.ds(pl.multiple_of(s2 * 8, 8), 8), :] = _pack(jnp.concatenate([lo, hi], axis=0).astype(BF16))
            return carry

        lax.fori_loop(0, n_seg // 2, last_rows, 0, unroll=4)

        with scope('ahead'):
            flipped = 0
            for t, nf in enumerate(FLIPS):
                for d in range(flipped, flipped + nf):
                    cp_w[d].wait()
                assert DW * (flipped + nf) >= CW * UA * (t + 1)
                for n in range(t * UA, (t + 1) * UA):
                    i, c0 = n // NC, (n % NC) * CW
                    pre_s[n] = lax.dot_general(_unpack(xl_s[...]), stage[i, c0:c0 + CW, :], NT,
                                               preferred_element_type=F32)
                for d in range(flipped, flipped + nf):
                    i, c0 = d // ND, (d % ND) * DW
                    w_s[i, :, c0:c0 + DW] = _pack(stage[i, c0:c0 + DW, :].T)
                flipped += nf
        for cp in cp_w[3 * ND:]:
            cp.wait()

        mem_s[...] = mem0_ref[...].astype(F32)
        gate = gate_ref[...].astype(F32).reshape(1, D)

        def step(s, carry):
            row = lax.broadcasted_iota(I32, (L, LANES), 0)
            lane = lax.broadcasted_iota(I32, (L, LANES), 1)
            first = lane < L
            second = (lane >= L) & (lane < 2 * L)
            visible = (row < M) | (row >= jnp.where(first, lane, lane - L))
            lo_half = lane < LANES // 2
            zeros = jnp.zeros((L, LANES), F32)
            r0 = pl.multiple_of(s * seg, seg)
            p0 = pl.multiple_of(s * 8, 8)
            xs = x_s[pl.ds(r0, seg), :].astype(F32)
            h = jnp.concatenate([mem_s[...], xs], axis=0)

            def blockdiag(t0, t1, t2):
                top = jnp.concatenate([t0, jnp.where(lo_half, t1, 0.0), zeros], axis=1)
                bot = jnp.concatenate([zeros, jnp.where(lo_half, 0.0, t1), t2], axis=1)
                return jnp.concatenate([top, bot], axis=0).astype(BF16)

            def project(i, G, j):
                c0 = (3 * G + j) * CW
                w = _unpack(w_s[i, :, c0:c0 + CW])
                n = i * NC + c0 // CW
                if n < NPRE:
                    y = jnp.dot(h[0:L - 8], w, preferred_element_type=F32)
                    y = jnp.concatenate([y, pre_s[n, pl.ds(p0, 8), :]], axis=0)
                else:
                    y = jnp.dot(h, w, preferred_element_type=F32)
                return [y[:, t * LANES:(t + 1) * LANES] for t in range(4)]

            def softmax(sc):
                sc = jnp.concatenate([sc, jnp.zeros((L, LANES - 2 * L), F32)], axis=1)
                sc = jnp.where(visible, sc * scale, -1e9)
                m1 = jnp.max(jnp.where(first, sc, -jnp.inf), axis=1, keepdims=True)
                m2 = jnp.max(jnp.where(second, sc, -jnp.inf), axis=1, keepdims=True)
                e = jnp.exp(sc - jnp.where(first, m1, m2))
                l1 = jnp.sum(jnp.where(first, e, 0.0), axis=1, keepdims=True)
                l2 = jnp.sum(jnp.where(second, e, 0.0), axis=1, keepdims=True)
                return (e / jnp.where(first, l1, l2))[:, 0:2 * L]

            qt, kt, vt, pt, ot = {}, {}, {}, {}, {}
            accs = [None] * (D // LANES)
            for op in make_sched(opts.get('sched', 2), NG):
                kind, G = op[0], int(op[1])
                if kind == 'q':
                    qt.setdefault(G, []).extend(project(0, G, int(op[2])))
                elif kind == 'k':
                    kt.setdefault(G, []).extend(project(1, G, int(op[2])))
                elif kind == 'v':
                    vt.setdefault(G, []).extend(project(2, G, int(op[2])))
                elif kind == 's':
                    pt[G] = [softmax(lax.dot_general(jnp.concatenate(qt[G][3 * p:3 * p + 3], axis=1),
                                                     blockdiag(*kt[G][3 * p:3 * p + 3]), NT,
                                                     preferred_element_type=F32)) for p in range(GP)]
                elif kind == 'p':
                    ot[G] = [jnp.dot(pt[G][p], blockdiag(*vt[G][3 * p:3 * p + 3]), preferred_element_type=F32)
                             for p in range(GP)]
                elif kind == 'o':
                    j = int(op[2])
                    for p in range(GP):
                        w0 = (G * GP + p) * PW
                        r = jnp.dot(ot[G][p], stage[3, w0:w0 + PW, j * LANES:(j + 1) * LANES],
                                    preferred_element_type=F32)
                        accs[j] = r if accs[j] is None else accs[j] + r
            acc = jnp.concatenate(accs, axis=1)

            mem_s[...] = acc[0:M]
            g = jax.nn.sigmoid(jnp.sum(xs * gate, axis=1, keepdims=True))
            b = xs * v_s[pl.ds(r0, seg), :].astype(F32)
            out_s[pl.ds(r0, seg), :] = (g * acc[M:L] + (1.0 - g) * b).astype(BF16)
            pltpu.make_async_copy(out_s.at[pl.ds(r0, seg), :], out_hbm.at[pl.ds(r0, seg), :], sem_out.at[0]).start()
            return carry

        nsteps = opts.get('nsteps', n_seg)
        with scope('main'):
            lax.fori_loop(0, nsteps, step, 0, unroll=opts.get('unroll', 2))
        pltpu.make_async_copy(out_s.at[pl.ds(0, nsteps * seg), :], out_hbm.at[pl.ds(0, nsteps * seg), :],
                              sem_out.at[0]).wait()

    scratch = [
        pltpu.VMEM((S, D), BF16),
        pltpu.VMEM((S, D), BF16),
        pltpu.VMEM((S, D), BF16),
        pltpu.VMEM((D, S), BF16),
        pltpu.VMEM((4, HD, D), BF16),
        pltpu.VMEM((3, D // 2, HD), I32),
        pltpu.VMEM(((ks + 1) // 2, 8, D), F32),
        pltpu.VMEM((nb, 2 * C, D), F32),
        pltpu.VMEM((nb, 2 * C, D), F32),
        pltpu.VMEM((nb, 2 * C, D), F32),
        pltpu.VMEM((n_seg * 4, D), I32),
        pltpu.VMEM((NPRE, n_seg * 8, CW), F32),
        pltpu.VMEM((M, D), F32),
        pltpu.SemaphoreType.DMA((1,)),
        pltpu.SemaphoreType.DMA((len(FPS) - 1,)),
        pltpu.SemaphoreType.DMA((2 * KP,)),
        pltpu.SemaphoreType.DMA((4 * ND,)),
        pltpu.SemaphoreType.DMA((1,)),
    ]
    return kernel, scratch


_OPTS = {'ua':4,'flips':(2,3,3,4)}


@functools.partial(jax.jit, static_argnames=("A_seg_len",))
def pallas_gated_mix__memory_aug_recurrent_mem_tr__ssm_conv_h3__prompt_kernel(
    A_x, A_mem0, A_Wq, A_Wk, A_Wv, A_Wo, A_seg_len, B_q, B_k, B_v, B_shift_k, B_ssm_k, B_ssm_D, gate_w,
):
    opts = _OPTS
    B, S, D = A_x.shape
    H, Dh = A_Wq.shape[1], A_Wq.shape[2]
    M = A_mem0.shape[1]
    C = 256
    kernel, scratch = make_kernel(S, D, H, Dh, M, int(A_seg_len), B_shift_k.shape[1], C, opts)
    wt = lambda w: jnp.transpose(w, (1, 2, 0)).reshape(H * Dh, D)
    hbm = pl.BlockSpec(memory_space=pl.ANY)
    vmem = pl.BlockSpec(memory_space=pltpu.VMEM)
    out = pl.pallas_call(
        kernel,
        out_shape=jax.ShapeDtypeStruct((S, D), BF16),
        in_specs=[hbm, vmem, hbm, hbm, hbm, hbm, hbm, hbm, vmem, hbm, vmem, vmem, vmem, vmem, vmem],
        out_specs=hbm,
        scratch_shapes=scratch,
        compiler_params=pltpu.CompilerParams(vmem_limit_bytes=126 * 1024 * 1024, **opts.get('cp', {})),
    )(A_x.reshape(S, D), A_mem0.reshape(M, D), wt(A_Wq), wt(A_Wk), wt(A_Wv), A_Wo.reshape(H * Dh, D),
      B_k.reshape(S, D), B_v.reshape(S, D), B_shift_k.T, B_ssm_k, B_ssm_D, gate_w, *_dft_consts(C))
    return out.reshape(B, S, D)
```

```python
import functools

import jax
import jax.numpy as jnp
import numpy as np
from jax import lax
from jax.experimental import pallas as pl
from jax.experimental.pallas import tpu as pltpu

F32 = jnp.float32
BF16 = jnp.bfloat16
I32 = jnp.int32
NT = (((1,), (1,)), ((), ()))
LANES = 128
CHUNK = 256


def _pack_rows(a):
    u = np.ascontiguousarray(a.astype(jnp.bfloat16)).view(np.uint16).astype(np.uint32)
    return (u[0::2] | (u[1::2] << 16)).view(np.int32)


def _dft_consts(C):
    k = np.concatenate([np.arange(0, C, 2), np.arange(1, C, 2)])[:, None]
    n = np.arange(C)[None, :]
    ang = np.pi * (((2 * k + 1) * n) % (4 * C)) / (2 * C)
    full = np.concatenate([np.cos(ang), -np.sin(ang)], axis=0)
    u = np.arange(C // 2)[None, :]
    ang = np.pi * (((2 * k + 1) * (2 * u + 1)) % (8 * C)) / (4 * C)
    half = np.concatenate([np.cos(ang), -np.sin(ang)], axis=0)
    inv = half.T / C
    return _pack_rows(full), _pack_rows(half), _pack_rows(inv)


def _pack(a):
    return pltpu.bitcast(a, I32)


def _unpack(a):
    return pltpu.bitcast(a, BF16)


def _reverse_rows(a):
    idx = 7 - lax.broadcasted_iota(I32, (8, a.shape[1]), 0)
    return jnp.concatenate(
        [jnp.take_along_axis(a[r:r + 8], idx, axis=0) for r in range(a.shape[0] - 8, -8, -8)], axis=0)


def _make_kernel(S, D, H, Dh, M, seg, ks):
    C = CHUNK
    nb = S // C
    n_seg = S // seg
    L = M + seg
    HD = H * Dh
    PW = 2 * Dh
    scale = float(Dh) ** -0.5
    CW = 4 * LANES
    NC = HD // CW
    GP = 4
    NG = H // 2 // GP
    DW = 3 * CW
    ND = HD // DW
    ROUNDS = 4
    UA = 4
    UF = 3 * ND // ROUNDS
    NPRE = UA * ROUNDS
    FP = (0, nb // 4, nb)
    KP = 2
    assert PW == 3 * LANES and 2 * L <= LANES and M == 8 and seg % 16 == 0 and n_seg % 2 == 0
    assert D % LANES == 0 and S % (4 * C) == 0 and H % (2 * GP) == 0
    assert UF * ROUNDS == 3 * ND and UF * DW >= UA * CW

    def kernel(x_hbm, wq_hbm, wk_hbm, wv_hbm, wo_hbm, k_hbm, v_hbm, f_hbm,
               full_hbm, half_hbm, inv_hbm, shift_hbm, dvec_hbm, gate_hbm, mem0_hbm,
               out_hbm,
               full_s, half_s, inv_s, shift_s, dvec_s, gate_s, mem0_s,
               x_s, k_s, v_s, f_s, wt_s, w_s, tail_s, X_s, F_s, W_s, xl_s, pre_s, mem_s,
               sem_small, sem_x, sem_f, sem_kv, sem_w, sem_out):
        out_s = k_s

        cp_small = [pltpu.make_async_copy(src, dst, sem_small.at[e]) for e, (src, dst) in enumerate((
            (full_hbm, full_s), (half_hbm, half_s), (inv_hbm, inv_s), (shift_hbm, shift_s),
            (dvec_hbm, dvec_s), (gate_hbm, gate_s), (mem0_hbm, mem0_s)))]
        cp_x = pltpu.make_async_copy(x_hbm, x_s, sem_x.at[0])
        cp_f = [pltpu.make_async_copy(f_hbm.at[:, pl.ds(a * C, (b - a) * C)],
                                      f_s.at[:, pl.ds(a * C, (b - a) * C)], sem_f.at[p])
                for p, (a, b) in enumerate(zip(FP[:-1], FP[1:]))]
        cp_kv = [[pltpu.make_async_copy(src.at[pl.ds(p * S // KP, S // KP), :],
                                        dst.at[pl.ds(p * S // KP, S // KP), :], sem_kv.at[2 * p + e])
                  for e, (src, dst) in enumerate(((k_hbm, k_s), (v_hbm, v_s)))] for p in range(KP)]
        cp_w = [pltpu.make_async_copy(w.at[pl.ds(d * DW, DW), :], wt_s.at[pl.ds(i * HD + d * DW, DW), :],
                                      sem_w.at[i * ND + d])
                for i, w in enumerate((wq_hbm, wk_hbm, wv_hbm, wo_hbm)) for d in range(ND)]
        loads = cp_small[:1] + cp_f + cp_small[1:] + sum(cp_kv, []) + [cp_x] + cp_w

        def issue(n, carry):
            for idx, cp in enumerate(loads):
                pl.when(n == idx)(cp.start)
            return carry

        lax.fori_loop(0, len(loads), issue, 0)

        def filt(m, carry):
            c0 = pl.multiple_of(m * C, C)
            F_s[m] = lax.dot_general(_unpack(full_s[...]), f_s[:, pl.ds(c0, C)], NT, preferred_element_type=F32)
            return carry

        cp_small[0].wait()
        for p, (a, b) in enumerate(zip(FP[:-1], FP[1:])):
            cp_f[p].wait()
            lax.fori_loop(a, b, filt, 0, unroll=2)

        def delay(a, n, slot):
            tail = tail_s[slot]
            tail_s[slot] = a[a.shape[0] - 8:]
            rolled = [pltpu.roll(g, n, 0) for g in [tail] + [a[r:r + 8] for r in range(0, a.shape[0], 8)]]
            early = lax.broadcasted_iota(I32, tail.shape, 0) < n
            return jnp.concatenate([jnp.where(early, p, c) for p, c in zip(rolled[:-1], rolled[1:])], axis=0)

        def sig(j, carry):
            r0 = pl.multiple_of(j * C, C)
            taps = shift_s[...].astype(F32)
            kc = k_s[pl.ds(r0, C), :].astype(F32)
            k1 = delay(kc, 1, 0)
            acc = None
            for p in range((ks + 1) // 2):
                pair = kc * taps[2 * p:2 * p + 1, :]
                if 2 * p + 1 < ks:
                    pair = pair + k1 * taps[2 * p + 1:2 * p + 2, :]
                acc = pair if p == 0 else acc + delay(pair, 2 * p, p)
            kv = acc * v_s[pl.ds(r0, C), :].astype(F32)
            v_s[pl.ds(r0, C), :] = kv.astype(BF16)
            up, down = kv[C // 2:C], _reverse_rows(kv[0:C // 2])
            X_s[j, 0:C] = jnp.dot(_unpack(half_s[0:C // 2, :]), (up + down).astype(BF16),
                                  preferred_element_type=F32)
            X_s[j, C:2 * C] = jnp.dot(_unpack(half_s[C // 2:C, :]), (up - down).astype(BF16),
                                      preferred_element_type=F32)
            return carry

        tail_s[...] = jnp.zeros(tail_s.shape, F32)
        for cp in cp_small[1:]:
            cp.wait()
        for p in range(KP):
            for cp in cp_kv[p]:
                cp.wait()
            lax.fori_loop(p * nb // KP, (p + 1) * nb // KP, sig, 0, unroll=2)

        def freq(r, carry, odd):
            re = pl.ds(pl.multiple_of(r * 8, 8), 8)
            im = pl.ds(pl.multiple_of(C + r * 8, 8), 8)
            for c in range(D // LANES):
                cs = slice(c * LANES, (c + 1) * LANES)
                xr = [X_s[j, re, cs] for j in range(nb)]
                xi = [X_s[j, im, cs] for j in range(nb)]
                fr = [F_s[j, re, cs] for j in range(nb)]
                fi = [F_s[j, im, cs] for j in range(nb)]
                if odd:
                    gr = [fr[0]] + [fr[m] + fi[m - 1] for m in range(1, nb)]
                    gi = [fi[0]] + [fi[m] - fr[m - 1] for m in range(1, nb)]
                else:
                    gr = [fr[0]] + [fr[m] - fi[m - 1] for m in range(1, nb)]
                    gi = [fi[0]] + [fi[m] + fr[m - 1] for m in range(1, nb)]
                xs = [a + b for a, b in zip(xr, xi)]
                gd = [b - a for a, b in zip(gr, gi)]
                gs = [a + b for a, b in zip(gr, gi)]
                for i in range(nb):
                    k1 = k2 = k3 = None
                    for j in range(i + 1):
                        t1, t2, t3 = gr[i - j] * xs[j], xr[j] * gd[i - j], xi[j] * gs[i - j]
                        k1, k2, k3 = (t1, t2, t3) if j == 0 else (k1 + t1, k2 + t2, k3 + t3)
                    W_s[i, re, cs] = k1 - k3
                    W_s[i, im, cs] = k1 + k2
            return carry

        lax.fori_loop(0, C // 16, functools.partial(freq, odd=False), 0)
        lax.fori_loop(C // 16, C // 8, functools.partial(freq, odd=True), 0)

        def inverse(i, carry):
            r0 = pl.multiple_of(i * C, C)
            even = jnp.dot(_unpack(inv_s[:, 0:C]), W_s[i, 0:C].astype(BF16), preferred_element_type=F32)
            odd = jnp.dot(_unpack(inv_s[:, C:2 * C]), W_s[i, C:2 * C].astype(BF16), preferred_element_type=F32)
            y = jnp.concatenate([_reverse_rows(even - odd), even + odd], axis=0)
            dvec = dvec_s[...].astype(F32).reshape(1, D)
            v_s[pl.ds(r0, C), :] = (y + v_s[pl.ds(r0, C), :].astype(F32) * dvec).astype(BF16)
            return carry

        lax.fori_loop(0, nb, inverse, 0, unroll=2)

        cp_x.wait()

        def last_rows(s2, carry):
            r0 = pl.multiple_of(s2 * 2 * seg, 2 * seg)
            lo = x_s[pl.ds(r0 + seg - 16, 16), :].astype(F32)[8:16]
            hi = x_s[pl.ds(r0 + 2 * seg - 16, 16), :].astype(F32)[8:16]
            xl_s[pl.ds(pl.multiple_of(s2 * 8, 8), 8), :] = _pack(jnp.concatenate([lo, hi], axis=0).astype(BF16))
            return carry

        lax.fori_loop(0, n_seg // 2, last_rows, 0, unroll=4)

        def ahead(t, carry):
            blocks = [pl.ds(pl.multiple_of((t * UF + e) * DW, DW), DW) for e in range(UF)]
            for e, rows in enumerate(blocks):
                pltpu.make_async_copy(wt_s.at[rows, :], wt_s.at[rows, :], sem_w.at[t * UF + e]).wait()
            for e in range(UA):
                n = t * UA + e
                pre_s[n] = lax.dot_general(_unpack(xl_s[...]), wt_s[pl.ds(pl.multiple_of(n * CW, CW), CW), :], NT,
                                           preferred_element_type=F32)
            for rows in blocks:
                w_s[:, rows] = _pack(wt_s[rows, :].T)
            return carry

        lax.fori_loop(0, ROUNDS, ahead, 0)
        for cp in cp_w[3 * ND:]:
            cp.wait()

        mem_s[...] = mem0_s[...].astype(F32)
        gate = gate_s[...].astype(F32).reshape(1, D)

        def step(s, carry):
            row = lax.broadcasted_iota(I32, (L, LANES), 0)
            lane = lax.broadcasted_iota(I32, (L, LANES), 1)
            first = lane < L
            real = lane < 2 * L
            visible = real & ((row < M) | (row >= jnp.where(first, lane, lane - L)))
            fill = jnp.where(real, -1e9, -jnp.inf)
            lo_half = lane < LANES // 2
            zeros = jnp.zeros((L, LANES), F32)
            rows = pl.ds(pl.multiple_of(s * seg, seg), seg)
            xs = x_s[rows, :].astype(F32)
            h = jnp.concatenate([mem_s[...], xs], axis=0)

            def project(i, G, part=range(3)):
                tiles = []
                for n in [i * NC + 3 * G + j for j in part]:
                    w = _unpack(w_s[:, n * CW:(n + 1) * CW])
                    if n < NPRE:
                        y = jnp.dot(h[0:L - 8], w, preferred_element_type=F32)
                        y = jnp.concatenate([y, pre_s[n, pl.ds(pl.multiple_of(s * 8, 8), 8), :]], axis=0)
                    else:
                        y = jnp.dot(h, w, preferred_element_type=F32)
                    tiles += [y[:, t * LANES:(t + 1) * LANES] for t in range(CW // LANES)]
                return tiles

            def blockdiag(t0, t1, t2):
                top = jnp.concatenate([t0, jnp.where(lo_half, t1, 0.0), zeros], axis=1)
                bot = jnp.concatenate([zeros, jnp.where(lo_half, 0.0, t1), t2], axis=1)
                return jnp.concatenate([top, bot], axis=0).astype(BF16)

            def attention_weights(q, k):
                sc = lax.dot_general(jnp.concatenate(q, axis=1), blockdiag(*k), NT, preferred_element_type=F32)
                sc = jnp.concatenate([sc, jnp.zeros((L, LANES - 2 * L), F32)], axis=1)
                sc = jnp.where(visible, sc * scale, fill)
                m1 = jnp.max(jnp.where(first, sc, -jnp.inf), axis=1, keepdims=True)
                m2 = jnp.max(jnp.where(first, -jnp.inf, sc), axis=1, keepdims=True)
                e = jnp.exp(sc - jnp.where(first, m1, m2))
                l1 = jnp.sum(jnp.where(first, e, 0.0), axis=1, keepdims=True)
                l2 = jnp.sum(jnp.where(first, 0.0, e), axis=1, keepdims=True)
                return (e / jnp.where(first, l1, l2))[:, 0:2 * L]

            def mix_values(p, v):
                return [jnp.dot(p[e], blockdiag(*v[3 * e:3 * e + 3]), preferred_element_type=F32) for e in range(GP)]

            acc = [None] * (D // LANES)

            def project_out(o, G):
                for j in range(D // LANES):
                    for p in range(GP):
                        w0 = 3 * HD + (G * GP + p) * PW
                        r = jnp.dot(o[p], wt_s[w0:w0 + PW, j * LANES:(j + 1) * LANES], preferred_element_type=F32)
                        acc[j] = r if acc[j] is None else acc[j] + r

            pending = None
            for G in range(NG):
                k = project(1, G)
                o = mix_values(*pending) if pending else None
                q = project(0, G)
                v = project(2, G, (0,))
                p = [attention_weights(q[3 * e:3 * e + 3], k[3 * e:3 * e + 3]) for e in range(GP)]
                pending = (p, v + project(2, G, (1, 2)))
                if o:
                    project_out(o, G - 1)
            project_out(mix_values(*pending), NG - 1)
            a = jnp.concatenate(acc, axis=1)

            mem_s[...] = a[0:M]
            g = jax.nn.sigmoid(jnp.sum(xs * gate, axis=1, keepdims=True))
            b = xs * v_s[rows, :].astype(F32)
            out_s[rows, :] = (g * a[M:L] + (1.0 - g) * b).astype(BF16)
            pltpu.make_async_copy(out_s.at[rows, :], out_hbm.at[rows, :], sem_out.at[0]).start()
            return carry

        lax.fori_loop(0, n_seg, step, 0, unroll=4)
        pltpu.make_async_copy(out_s, out_hbm, sem_out.at[0]).wait()

    scratch = [
        pltpu.VMEM((C, C), I32),
        pltpu.VMEM((C, C // 2), I32),
        pltpu.VMEM((C // 4, 2 * C), I32),
        pltpu.VMEM((ks, D), BF16),
        pltpu.VMEM((D,), BF16),
        pltpu.VMEM((D,), BF16),
        pltpu.VMEM((M, D), BF16),
        pltpu.VMEM((S, D), BF16),
        pltpu.VMEM((S, D), BF16),
        pltpu.VMEM((S, D), BF16),
        pltpu.VMEM((D, S), BF16),
        pltpu.VMEM((4 * HD, D), BF16),
        pltpu.VMEM((D // 2, 3 * HD), I32),
        pltpu.VMEM(((ks + 1) // 2, 8, D), F32),
        pltpu.VMEM((nb, 2 * C, D), F32),
        pltpu.VMEM((nb, 2 * C, D), F32),
        pltpu.VMEM((nb, 2 * C, D), F32),
        pltpu.VMEM((n_seg * 4, D), I32),
        pltpu.VMEM((NPRE, n_seg * 8, CW), F32),
        pltpu.VMEM((M, D), F32),
        pltpu.SemaphoreType.DMA((7,)),
        pltpu.SemaphoreType.DMA((1,)),
        pltpu.SemaphoreType.DMA((len(FP) - 1,)),
        pltpu.SemaphoreType.DMA((2 * KP,)),
        pltpu.SemaphoreType.DMA((4 * ND,)),
        pltpu.SemaphoreType.DMA((1,)),
    ]
    return kernel, scratch


@functools.partial(jax.jit, static_argnames=("A_seg_len",))
def pallas_gated_mix__memory_aug_recurrent_mem_tr__ssm_conv_h3__prompt_kernel(
    A_x: jax.Array,
    A_mem0: jax.Array,
    A_Wq: jax.Array,
    A_Wk: jax.Array,
    A_Wv: jax.Array,
    A_Wo: jax.Array,
    A_seg_len: int,
    B_q: jax.Array,
    B_k: jax.Array,
    B_v: jax.Array,
    B_shift_k: jax.Array,
    B_ssm_k: jax.Array,
    B_ssm_D: jax.Array,
    gate_w: jax.Array,
):
    del B_q
    B, S, D = A_x.shape
    H, Dh = A_Wq.shape[1], A_Wq.shape[2]
    M = A_mem0.shape[1]
    assert B == 1
    kernel, scratch = _make_kernel(S, D, H, Dh, M, int(A_seg_len), B_shift_k.shape[1])

    def transposed(w):
        return jnp.transpose(w, (1, 2, 0)).reshape(H * Dh, D)

    args = (A_x.reshape(S, D), transposed(A_Wq), transposed(A_Wk), transposed(A_Wv), A_Wo.reshape(H * Dh, D),
            B_k.reshape(S, D), B_v.reshape(S, D), B_ssm_k,
            *_dft_consts(CHUNK), B_shift_k.T, B_ssm_D, gate_w, A_mem0.reshape(M, D))
    hbm = pl.BlockSpec(memory_space=pl.ANY)
    out = pl.pallas_call(
        kernel,
        out_shape=jax.ShapeDtypeStruct((S, D), BF16),
        in_specs=[hbm] * len(args),
        out_specs=hbm,
        scratch_shapes=scratch,
        compiler_params=pltpu.CompilerParams(vmem_limit_bytes=124 * 1024 * 1024),
    )(*args)
    return out.reshape(B, S, D)
```

```python
import functools

import jax
import jax.numpy as jnp
import numpy as np
from jax import lax
from jax.experimental import pallas as pl
from jax.experimental.pallas import tpu as pltpu

F32 = jnp.float32
BF16 = jnp.bfloat16
I32 = jnp.int32
NT = (((1,), (1,)), ((), ()))
LANES = 128
CHUNK = 256


def _pack_rows(a):
    u = np.ascontiguousarray(a.astype(jnp.bfloat16)).view(np.uint16).astype(np.uint32)
    return (u[0::2] | (u[1::2] << 16)).view(np.int32)


def _dft_consts(C):
    k = np.concatenate([np.arange(0, C, 2), np.arange(1, C, 2)])[:, None]
    n = np.arange(C)[None, :]
    ang = np.pi * (((2 * k + 1) * n) % (4 * C)) / (2 * C)
    full = np.concatenate([np.cos(ang), -np.sin(ang)], axis=0)
    u = np.arange(C // 2)[None, :]
    ang = np.pi * (((2 * k + 1) * (2 * u + 1)) % (8 * C)) / (4 * C)
    half = np.concatenate([np.cos(ang), -np.sin(ang)], axis=0)
    inv = half.T / C
    return _pack_rows(full), _pack_rows(half), _pack_rows(inv)


def _pack(a):
    return pltpu.bitcast(a, I32)


def _unpack(a):
    return pltpu.bitcast(a, BF16)


def _reverse_rows(a):
    idx = 7 - lax.broadcasted_iota(I32, (8, a.shape[1]), 0)
    return jnp.concatenate(
        [jnp.take_along_axis(a[r:r + 8], idx, axis=0) for r in range(a.shape[0] - 8, -8, -8)], axis=0)


def _make_kernel(S, D, H, Dh, M, seg, ks):
    C = CHUNK
    nb = S // C
    n_seg = S // seg
    L = M + seg
    HD = H * Dh
    PW = 2 * Dh
    scale = float(Dh) ** -0.5
    CW = 4 * LANES
    NC = HD // CW
    GP = 4
    NG = H // 2 // GP
    DW = 3 * CW
    ND = HD // DW
    ROUNDS = 4
    UA = 4
    UF = 3 * ND // ROUNDS
    NPRE = UA * ROUNDS
    FP = (0, nb // 4, nb)
    US = 4
    KP = 2
    assert PW == 3 * LANES and 2 * L <= LANES and M == 8 and seg % 16 == 0 and n_seg % US == 0
    assert US % 2 == 0 and n_seg >= 2 * US
    assert D % LANES == 0 and S % (4 * C) == 0 and H % (2 * GP) == 0
    assert UF * ROUNDS == 3 * ND and UF * DW >= UA * CW

    def kernel(x_hbm, xseg_hbm, wq_hbm, wk_hbm, wv_hbm, wo_hbm, k_hbm, v_hbm, f_hbm,
               full_hbm, half_hbm, inv_hbm, shift_hbm, dvec_hbm, gate_hbm, mem0_hbm,
               out_hbm,
               full_s, half_s, inv_s, shift_s, dvec_s, gate_s, mem0_s,
               x_s, xe_s, k_s, v_s, f_s, wt_s, w_s, tail_s, X_s, F_s, W_s, xl_s, pre_s, mem_s,
               sem_small, sem_x, sem_f, sem_kv, sem_w, sem_out):
        out_s = k_s

        cp_small = [pltpu.make_async_copy(src, dst, sem_small.at[e]) for e, (src, dst) in enumerate((
            (full_hbm, full_s), (half_hbm, half_s), (inv_hbm, inv_s), (shift_hbm, shift_s),
            (dvec_hbm, dvec_s), (gate_hbm, gate_s), (mem0_hbm, mem0_s)))]
        cp_xe = pltpu.make_async_copy(xseg_hbm.at[:, pl.ds(seg - 8, 8), :], xe_s, sem_x.at[0])
        cp_x = [pltpu.make_async_copy(x_hbm.at[pl.ds(a, b - a), :], x_s.at[pl.ds(a, b - a), :], sem_x.at[1 + e])
                for e, (a, b) in enumerate(((0, US * seg), (US * seg, S)))]
        cp_f = [pltpu.make_async_copy(f_hbm.at[:, pl.ds(a * C, (b - a) * C)],
                                      f_s.at[:, pl.ds(a * C, (b - a) * C)], sem_f.at[p])
                for p, (a, b) in enumerate(zip(FP[:-1], FP[1:]))]
        cp_kv = [[pltpu.make_async_copy(src.at[pl.ds(p * S // KP, S // KP), :],
                                        dst.at[pl.ds(p * S // KP, S // KP), :], sem_kv.at[2 * p + e])
                  for e, (src, dst) in enumerate(((k_hbm, k_s), (v_hbm, v_s)))] for p in range(KP)]
        cp_w = [pltpu.make_async_copy(w.at[pl.ds(d * DW, DW), :], wt_s.at[pl.ds(i * HD + d * DW, DW), :],
                                      sem_w.at[i * ND + d])
                for i, w in enumerate((wq_hbm, wk_hbm, wv_hbm, wo_hbm)) for d in range(ND)]
        loads = cp_small[:1] + cp_f + cp_small[1:] + sum(cp_kv, []) + [cp_xe, cp_x[0]] + cp_w + [cp_x[1]]

        def issue(n, carry):
            for idx, cp in enumerate(loads):
                pl.when(n == idx)(cp.start)
            return carry

        lax.fori_loop(0, len(loads), issue, 0)

        def filt(m, carry):
            c0 = pl.multiple_of(m * C, C)
            F_s[m] = lax.dot_general(_unpack(full_s[...]), f_s[:, pl.ds(c0, C)], NT, preferred_element_type=F32)
            return carry

        cp_small[0].wait()
        for p, (a, b) in enumerate(zip(FP[:-1], FP[1:])):
            cp_f[p].wait()
            lax.fori_loop(a, b, filt, 0, unroll=min(3, b - a))

        def delay(a, n, slot):
            tail = tail_s[slot]
            tail_s[slot] = a[a.shape[0] - 8:]
            rolled = [pltpu.roll(g, n, 0) for g in [tail] + [a[r:r + 8] for r in range(0, a.shape[0], 8)]]
            early = lax.broadcasted_iota(I32, tail.shape, 0) < n
            return jnp.concatenate([jnp.where(early, p, c) for p, c in zip(rolled[:-1], rolled[1:])], axis=0)

        def sig(j, carry):
            r0 = pl.multiple_of(j * C, C)
            taps = shift_s[...].astype(F32)
            kc = k_s[pl.ds(r0, C), :].astype(F32)
            k1 = delay(kc, 1, 0)
            acc = None
            for p in range((ks + 1) // 2):
                pair = kc * taps[2 * p:2 * p + 1, :]
                if 2 * p + 1 < ks:
                    pair = pair + k1 * taps[2 * p + 1:2 * p + 2, :]
                acc = pair if p == 0 else acc + delay(pair, 2 * p, p)
            kv = acc * v_s[pl.ds(r0, C), :].astype(F32)
            v_s[pl.ds(r0, C), :] = kv.astype(BF16)
            up, down = kv[C // 2:C], _reverse_rows(kv[0:C // 2])
            X_s[j, 0:C] = jnp.dot(_unpack(half_s[0:C // 2, :]), (up + down).astype(BF16),
                                  preferred_element_type=F32)
            X_s[j, C:2 * C] = jnp.dot(_unpack(half_s[C // 2:C, :]), (up - down).astype(BF16),
                                      preferred_element_type=F32)
            return carry

        tail_s[...] = jnp.zeros(tail_s.shape, F32)
        for cp in cp_small[1:]:
            cp.wait()
        for p in range(KP):
            for cp in cp_kv[p]:
                cp.wait()
            lax.fori_loop(p * nb // KP, (p + 1) * nb // KP, sig, 0, unroll=2)

        def freq(r, carry, odd):
            re = pl.ds(pl.multiple_of(r * 8, 8), 8)
            im = pl.ds(pl.multiple_of(C + r * 8, 8), 8)
            for c in range(D // LANES):
                cs = slice(c * LANES, (c + 1) * LANES)
                xr = [X_s[j, re, cs] for j in range(nb)]
                xi = [X_s[j, im, cs] for j in range(nb)]
                fr = [F_s[j, re, cs] for j in range(nb)]
                fi = [F_s[j, im, cs] for j in range(nb)]
                if odd:
                    gr = [fr[0]] + [fr[m] + fi[m - 1] for m in range(1, nb)]
                    gi = [fi[0]] + [fi[m] - fr[m - 1] for m in range(1, nb)]
                else:
                    gr = [fr[0]] + [fr[m] - fi[m - 1] for m in range(1, nb)]
                    gi = [fi[0]] + [fi[m] + fr[m - 1] for m in range(1, nb)]
                xs = [a + b for a, b in zip(xr, xi)]
                gd = [b - a for a, b in zip(gr, gi)]
                gs = [a + b for a, b in zip(gr, gi)]
                for i in range(nb):
                    k1 = k2 = k3 = None
                    for j in range(i + 1):
                        t1, t2, t3 = gr[i - j] * xs[j], xr[j] * gd[i - j], xi[j] * gs[i - j]
                        k1, k2, k3 = (t1, t2, t3) if j == 0 else (k1 + t1, k2 + t2, k3 + t3)
                    W_s[i, re, cs] = k1 - k3
                    W_s[i, im, cs] = k1 + k2
            return carry

        lax.fori_loop(0, C // 16, functools.partial(freq, odd=False), 0, unroll=2)
        lax.fori_loop(C // 16, C // 8, functools.partial(freq, odd=True), 0, unroll=2)

        def inverse(i, carry):
            r0 = pl.multiple_of(i * C, C)
            even = jnp.dot(_unpack(inv_s[:, 0:C]), W_s[i, 0:C].astype(BF16), preferred_element_type=F32)
            odd = jnp.dot(_unpack(inv_s[:, C:2 * C]), W_s[i, C:2 * C].astype(BF16), preferred_element_type=F32)
            y = jnp.concatenate([_reverse_rows(even - odd), even + odd], axis=0)
            dvec = dvec_s[...].astype(F32).reshape(1, D)
            v_s[pl.ds(r0, C), :] = (y + v_s[pl.ds(r0, C), :].astype(F32) * dvec).astype(BF16)
            return carry

        lax.fori_loop(0, nb, inverse, 0, unroll=4)

        cp_xe.wait()

        def last_rows(s2, carry):
            lo, hi = xe_s[2 * s2].astype(F32), xe_s[2 * s2 + 1].astype(F32)
            xl_s[pl.ds(pl.multiple_of(s2 * 8, 8), 8), :] = _pack(jnp.concatenate([lo, hi], axis=0).astype(BF16))
            return carry

        lax.fori_loop(0, n_seg // 2, last_rows, 0, unroll=4)

        def ahead(t, carry):
            blocks = [pl.ds(pl.multiple_of((t * UF + e) * DW, DW), DW) for e in range(UF)]
            for e, rows in enumerate(blocks):
                pltpu.make_async_copy(wt_s.at[rows, :], wt_s.at[rows, :], sem_w.at[t * UF + e]).wait()
            for e in range(UA):
                n = t * UA + e
                pre_s[n] = lax.dot_general(_unpack(xl_s[...]), wt_s[pl.ds(pl.multiple_of(n * CW, CW), CW), :], NT,
                                           preferred_element_type=F32)
            for rows in blocks:
                w_s[:, rows] = _pack(wt_s[rows, :].T)
            return carry

        lax.fori_loop(0, ROUNDS, ahead, 0)
        for cp in cp_w[3 * ND:] + cp_x[:1]:
            cp.wait()

        mem_s[...] = mem0_s[...].astype(F32)
        gate = gate_s[...].astype(F32).reshape(1, D)

        def step(s):
            row = lax.broadcasted_iota(I32, (L, LANES), 0)
            lane = lax.broadcasted_iota(I32, (L, LANES), 1)
            first = lane < L
            real = lane < 2 * L
            visible = real & ((row < M) | (row >= jnp.where(first, lane, lane - L)))
            fill = jnp.where(real, -1e9, -jnp.inf)
            lo_half = lane < LANES // 2
            zeros = jnp.zeros((L, LANES), F32)
            rows = pl.ds(pl.multiple_of(s * seg, seg), seg)
            xs = x_s[rows, :].astype(F32)
            h = jnp.concatenate([mem_s[...], xs], axis=0)

            def project(i, G, part=range(3)):
                tiles = []
                for n in [i * NC + 3 * G + j for j in part]:
                    w = _unpack(w_s[:, n * CW:(n + 1) * CW])
                    if n < NPRE:
                        y = jnp.dot(h[0:L - 8], w, preferred_element_type=F32)
                        y = jnp.concatenate([y, pre_s[n, pl.ds(pl.multiple_of(s * 8, 8), 8), :]], axis=0)
                    else:
                        y = jnp.dot(h, w, preferred_element_type=F32)
                    tiles += [y[:, t * LANES:(t + 1) * LANES] for t in range(CW // LANES)]
                return tiles

            def blockdiag(t0, t1, t2):
                top = jnp.concatenate([t0, jnp.where(lo_half, t1, 0.0), zeros], axis=1)
                bot = jnp.concatenate([zeros, jnp.where(lo_half, 0.0, t1), t2], axis=1)
                return jnp.concatenate([top, bot], axis=0).astype(BF16)

            def attention_weights(q, k):
                sc = lax.dot_general(jnp.concatenate(q, axis=1), blockdiag(*k), NT, preferred_element_type=F32)
                sc = jnp.concatenate([sc, jnp.zeros((L, LANES - 2 * L), F32)], axis=1)
                sc = jnp.where(visible, sc * scale, fill)
                m1 = jnp.max(jnp.where(first, sc, -jnp.inf), axis=1, keepdims=True)
                m2 = jnp.max(jnp.where(first, -jnp.inf, sc), axis=1, keepdims=True)
                e = jnp.exp(sc - jnp.where(first, m1, m2))
                l1 = jnp.sum(jnp.where(first, e, 0.0), axis=1, keepdims=True)
                l2 = jnp.sum(jnp.where(first, 0.0, e), axis=1, keepdims=True)
                return (e / jnp.where(first, l1, l2))[:, 0:2 * L]

            def mix_values(p, v):
                return [jnp.dot(p[e], blockdiag(*v[3 * e:3 * e + 3]), preferred_element_type=F32) for e in range(GP)]

            acc = [None] * (D // LANES)

            def project_out(o, G):
                for j in range(D // LANES):
                    for p in range(GP):
                        w0 = 3 * HD + (G * GP + p) * PW
                        r = jnp.dot(o[p], wt_s[w0:w0 + PW, j * LANES:(j + 1) * LANES], preferred_element_type=F32)
                        acc[j] = r if acc[j] is None else acc[j] + r

            pending = None
            for G in range(NG):
                k = project(1, G)
                o = mix_values(*pending) if pending else None
                q = project(0, G)
                v = project(2, G, (0,))
                p = [attention_weights(q[3 * e:3 * e + 3], k[3 * e:3 * e + 3]) for e in range(GP)]
                pending = (p, v + project(2, G, (1, 2)))
                if o:
                    project_out(o, G - 1)
            project_out(mix_values(*pending), NG - 1)
            a = jnp.concatenate(acc, axis=1)

            mem_s[...] = a[0:M]
            g = jax.nn.sigmoid(jnp.sum(xs * gate, axis=1, keepdims=True))
            b = xs * v_s[rows, :].astype(F32)
            out_s[rows, :] = (g * a[M:L] + (1.0 - g) * b).astype(BF16)
            pltpu.make_async_copy(out_s.at[rows, :], out_hbm.at[rows, :], sem_out.at[0]).start()

        def steps(t, carry):
            pl.when(t == 1)(cp_x[1].wait)
            for e in range(US):
                step(t * US + e)
            return carry

        lax.fori_loop(0, n_seg // US, steps, 0)
        pltpu.make_async_copy(out_s, out_hbm, sem_out.at[0]).wait()

    scratch = [
        pltpu.VMEM((C, C), I32),
        pltpu.VMEM((C, C // 2), I32),
        pltpu.VMEM((C // 4, 2 * C), I32),
        pltpu.VMEM((ks, D), BF16),
        pltpu.VMEM((D,), BF16),
        pltpu.VMEM((D,), BF16),
        pltpu.VMEM((M, D), BF16),
        pltpu.VMEM((S, D), BF16),
        pltpu.VMEM((n_seg, 8, D), BF16),
        pltpu.VMEM((S, D), BF16),
        pltpu.VMEM((S, D), BF16),
        pltpu.VMEM((D, S), BF16),
        pltpu.VMEM((4 * HD, D), BF16),
        pltpu.VMEM((D // 2, 3 * HD), I32),
        pltpu.VMEM(((ks + 1) // 2, 8, D), F32),
        pltpu.VMEM((nb, 2 * C, D), F32),
        pltpu.VMEM((nb, 2 * C, D), F32),
        pltpu.VMEM((nb, 2 * C, D), F32),
        pltpu.VMEM((n_seg * 4, D), I32),
        pltpu.VMEM((NPRE, n_seg * 8, CW), F32),
        pltpu.VMEM((M, D), F32),
        pltpu.SemaphoreType.DMA((7,)),
        pltpu.SemaphoreType.DMA((3,)),
        pltpu.SemaphoreType.DMA((len(FP) - 1,)),
        pltpu.SemaphoreType.DMA((2 * KP,)),
        pltpu.SemaphoreType.DMA((4 * ND,)),
        pltpu.SemaphoreType.DMA((1,)),
    ]
    return kernel, scratch


@functools.partial(jax.jit, static_argnames=("A_seg_len",))
def pallas_gated_mix__memory_aug_recurrent_mem_tr__ssm_conv_h3__prompt_kernel(
    A_x: jax.Array,
    A_mem0: jax.Array,
    A_Wq: jax.Array,
    A_Wk: jax.Array,
    A_Wv: jax.Array,
    A_Wo: jax.Array,
    A_seg_len: int,
    B_q: jax.Array,
    B_k: jax.Array,
    B_v: jax.Array,
    B_shift_k: jax.Array,
    B_ssm_k: jax.Array,
    B_ssm_D: jax.Array,
    gate_w: jax.Array,
):
    del B_q
    B, S, D = A_x.shape
    H, Dh = A_Wq.shape[1], A_Wq.shape[2]
    M = A_mem0.shape[1]
    assert B == 1
    seg = int(A_seg_len)
    kernel, scratch = _make_kernel(S, D, H, Dh, M, seg, B_shift_k.shape[1])

    def transposed(w):
        return jnp.transpose(w, (1, 2, 0)).reshape(H * Dh, D)

    args = (A_x.reshape(S, D), A_x.reshape(S // seg, seg, D), transposed(A_Wq), transposed(A_Wk), transposed(A_Wv), A_Wo.reshape(H * Dh, D),
            B_k.reshape(S, D), B_v.reshape(S, D), B_ssm_k,
            *_dft_consts(CHUNK), B_shift_k.T, B_ssm_D, gate_w, A_mem0.reshape(M, D))
    hbm = pl.BlockSpec(memory_space=pl.ANY)
    out = pl.pallas_call(
        kernel,
        out_shape=jax.ShapeDtypeStruct((S, D), BF16),
        in_specs=[hbm] * len(args),
        out_specs=hbm,
        scratch_shapes=scratch,
        compiler_params=pltpu.CompilerParams(vmem_limit_bytes=124 * 1024 * 1024),
    )(*args)
    return out.reshape(B, S, D)
```
